```python
import jax
import jax.numpy as jnp

def _softmax(x, axis=-1):
    return jax.nn.softmax(x, axis=axis)
def _gelu(x):
    return jax.nn.gelu(x, approximate=True)
def _silu(x):
    return jax.nn.silu(x)
def _sigmoid(x):
    return jax.nn.sigmoid(x)
def _layernorm(x, axis=-1, eps=1e-5):
    m = jnp.mean(x, axis=axis, keepdims=True)
    v = jnp.var(x, axis=axis, keepdims=True)
    return (x - m) / jnp.sqrt(v + eps)
def _scatter_add(tgt, idx, src, axis=0):
    return tgt.at[idx].add(src)
def _segment_sum(src, seg, n):
    return jax.ops.segment_sum(src, seg, n)
class _Rng:
    def __init__(self, key):
        self._k = key
    def _next(self):
        self._k, sub = jax.random.split(self._k)
        return sub
    def normal(self, shape):
        return jax.random.normal(self._next(), shape, dtype=jnp.bfloat16)
    def randint(self, lo, hi, shape):
        return jax.random.randint(self._next(), shape, lo, hi, dtype=jnp.int32)
    def uniform(self, shape, lo=0.0, hi=1.0):
        return jax.random.uniform(self._next(), shape, jnp.bfloat16, lo, hi)
    def permutation(self, n):
        return jax.random.permutation(self._next(), n)


kernel_name = 'recurrent_scan__sliding_block_cached__glu_gated_swiglu__decode'

def setup_inputs():
    _rng = _Rng(jax.random.key(int.from_bytes(__import__("os").urandom(4), "little")))
    _w = (lambda a: (lambda t: t.astype(jnp.bfloat16) if jnp.issubdtype(t.dtype, jnp.floating) else t)(jnp.asarray(a)))
    def _A_setup():
        B, Sq, D = 1, 1, 640
        Hq, Hkv, Sk, Dh = 32, 32, 32768, 192
        assert Hq % Hkv == 0, (Hq, Hkv)
        return {
            "x": _w((lambda *s: _rng.normal(s) * 0.05)(B, Sq, D)),
            "k_cache": _w((lambda *s: _rng.normal(s) * 0.05)(B, Hkv, Sk, Dh)),
            "v_cache": _w((lambda *s: _rng.normal(s) * 0.05)(B, Hkv, Sk, Dh)),
            "wq": _w((lambda *s: _rng.normal(s) * 0.05)(D, Hq * Dh) * (D ** -0.5)),
            "wo": _w((lambda *s: _rng.normal(s) * 0.05)(Hq * Dh, D) * ((Hq * Dh) ** -0.5)),
        }
    _A_in = _A_setup()

    def _B_setup():
        B, S, D, F = 1, 1, 640, 1536
        return {
            "x": _w((lambda *s: _rng.normal(s) * 0.05)(B, S, D)),
            "w1": _w((lambda *s: _rng.normal(s) * 0.05)(D, F) * (2.0 / D) ** 0.5),
            "w3": _w((lambda *s: _rng.normal(s) * 0.05)(D, F) * (2.0 / D) ** 0.5),
            "w2": _w((lambda *s: _rng.normal(s) * 0.05)(F, D) * (2.0 / F) ** 0.5),
        }
    _B_in = _B_setup()

    return {
        "A_x": _A_in["x"],
        "A_k_cache": _A_in["k_cache"],
        "A_v_cache": _A_in["v_cache"],
        "A_wq": _A_in["wq"],
        "A_wo": _A_in["wo"],
        "B_x": _B_in["x"],
        "B_w1": _B_in["w1"],
        "B_w3": _B_in["w3"],
        "B_w2": _B_in["w2"],
    }

def reference(A_x, A_k_cache, A_v_cache, A_wq, A_wo, B_x, B_w1, B_w3, B_w2):
    def _A_ref(x, k_cache, v_cache, wq, wo):
        B, Sq, D = x.shape
        Hq, Dh = 32, 192
        Hkv, Sk = k_cache.shape[1], k_cache.shape[2]
        W = min(4096, max(256, Sk // 4))
        rep = Hq // Hkv
        q = (lambda x, *d: x.transpose(*d))((x @ wq).reshape(B, Sq, Hq, Dh), 0, 2, 1, 3)
        k = jnp.repeat(k_cache[:, :, Sk - W:, :], rep, axis=1)
        v = jnp.repeat(v_cache[:, :, Sk - W:, :], rep, axis=1)
        scores = jnp.einsum("bhqd,bhkd->bhqk", q, k) * (Dh ** -0.5)
        p = _softmax(scores, axis=-1)
        o = jnp.einsum("bhqk,bhkd->bhqd", p, v)
        return (lambda x, *d: x.transpose(*d))(o, 0, 2, 1, 3).reshape(B, Sq, Hq * Dh) @ wo

    def _B_ref(x, w1, w3, w2):
        gate = jnp.einsum("bsd,df->bsf", x, w1)
        up = jnp.einsum("bsd,df->bsf", x, w3)
        h = _silu(gate) * up
        out = jnp.einsum("bsf,fd->bsd", h, w2)
        return out

    x = A_x
    xn = _layernorm(x, axis=-1)
    s = _A_ref(xn, A_k_cache, A_v_cache, A_wq, A_wo)
    g = _silu(_B_ref(xn, B_w1, B_w3, B_w2))
    return x + s * g
```

```python
import jax
import jax.numpy as jnp
from jax import lax
import jax.experimental.pallas as pl
import jax.experimental.pallas.tpu as pltpu

_HQ = 32
_DH = 192
_NB = 2
_EPS = 1e-5

_NN = (((1,), (0,)), ((), ()))
_NT = (((1,), (1,)), ((), ()))


def _silu(x):
    return x * jax.nn.sigmoid(x)


def _make_kernel(D, F, H, SK, W, wo_chunks):
    DH = _DH
    NP = H // 2
    PW = 2 * DH
    scale = DH ** -0.5

    def kernel(x_hbm, kt_hbm, vt_hbm, wq_hbm, wo_hbm, w1_hbm, w3_hbm, w2_hbm,
               out_ref,
               x_v, wq_v, wo_v, w1_v, w3_v, w2_v, kbuf, vbuf, q_scr, o_scr,
               sem_w, sem_k, sem_v, sem_o):
        def k_copy(h, slot):
            return pltpu.make_async_copy(
                kt_hbm.at[0, h, :, pl.ds(SK - W, W)], kbuf.at[slot], sem_k.at[slot])

        def v_copy(h, slot):
            return pltpu.make_async_copy(
                vt_hbm.at[0, h, :, pl.ds(SK - W, W)], vbuf.at[slot], sem_v.at[slot])

        def wo_copy(c):
            r0, r1 = wo_chunks[c]
            return pltpu.make_async_copy(
                wo_hbm.at[pl.ds(r0 * PW, (r1 - r0) * PW), :],
                wo_v.at[pl.ds(r0 * PW, (r1 - r0) * PW), :], sem_o.at[c])

        cx = pltpu.make_async_copy(x_hbm, x_v, sem_w.at[0])
        cq = pltpu.make_async_copy(wq_hbm, wq_v, sem_w.at[1])
        c1 = pltpu.make_async_copy(w1_hbm, w1_v, sem_w.at[2])
        c3 = pltpu.make_async_copy(w3_hbm, w3_v, sem_w.at[3])
        c2 = pltpu.make_async_copy(w2_hbm, w2_v, sem_w.at[4])

        cx.start()
        cq.start()
        c1.start()
        c3.start()
        c2.start()
        for s in range(_NB):
            k_copy(s, s).start()
            v_copy(s, s).start()

        cx.wait()
        x = x_v[...].astype(jnp.float32)
        mu = jnp.mean(x, axis=-1, keepdims=True)
        xc = x - mu
        var = jnp.mean(xc * xc, axis=-1, keepdims=True)
        xn = (xc / jnp.sqrt(var + _EPS)).astype(jnp.bfloat16)

        cq.wait()
        for p in range(NP):
            qp = lax.dot_general(xn, wq_v[:, p * PW:(p + 1) * PW], _NN,
                                 preferred_element_type=jnp.float32)
            q_scr[2 * p:2 * p + 1, :] = qp[:, :DH]
            q_scr[2 * p + 1:2 * p + 2, :] = qp[:, DH:]

        c1.wait()
        gate = lax.dot_general(xn, w1_v[...], _NN, preferred_element_type=jnp.float32)
        c3.wait()
        up = lax.dot_general(xn, w3_v[...], _NN, preferred_element_type=jnp.float32)
        hh = (_silu(gate) * up).astype(jnp.bfloat16)
        c2.wait()
        ffn = lax.dot_general(hh, w2_v[...], _NN, preferred_element_type=jnp.float32)
        g = _silu(ffn)

        def head(h, carry):
            slot = h % _NB
            q = q_scr[pl.ds(h, 1), :].astype(jnp.bfloat16)
            k_copy(h, slot).wait()
            s = lax.dot_general(q, kbuf[slot], _NN,
                                preferred_element_type=jnp.float32) * scale
            m = jnp.max(s, axis=-1, keepdims=True)
            p = jnp.exp(s - m)
            l = jnp.sum(p, axis=-1, keepdims=True)

            @pl.when(h + _NB < H)
            def _():
                k_copy(h + _NB, slot).start()

            v_copy(h, slot).wait()
            o = lax.dot_general(p.astype(jnp.bfloat16), vbuf[slot], _NT,
                                preferred_element_type=jnp.float32)
            o_scr[pl.ds(h, 1), :] = o / l

            @pl.when(h + _NB < H)
            def _():
                v_copy(h + _NB, slot).start()

            @pl.when(h + _NB == H - 1)
            def _():
                for c in range(len(wo_chunks)):
                    wo_copy(c).start()

            return carry

        lax.fori_loop(0, H, head, 0)

        acc = jnp.zeros((1, D), jnp.float32)
        for c in range(len(wo_chunks)):
            wo_copy(c).wait()
            r0, r1 = wo_chunks[c]
            for hh_ in range(2 * r0, 2 * r1):
                oh = o_scr[hh_:hh_ + 1, :].astype(jnp.bfloat16)
                acc = acc + lax.dot_general(
                    oh, wo_v[hh_ * DH:(hh_ + 1) * DH, :], _NN,
                    preferred_element_type=jnp.float32)

        out_ref[...] = (x + acc * g).astype(out_ref.dtype)

    return kernel


@jax.jit
def pallas_recurrent_scan__sliding_block_cached__glu_gated_swiglu__decode_kernel(
    A_x: jax.Array,
    A_k_cache: jax.Array,
    A_v_cache: jax.Array,
    A_wq: jax.Array,
    A_wo: jax.Array,
    B_x: jax.Array,
    B_w1: jax.Array,
    B_w3: jax.Array,
    B_w2: jax.Array,
):
    B, Sq, D = A_x.shape
    _, H, SK, DH = A_k_cache.shape
    F = B_w1.shape[1]
    assert B == 1 and Sq == 1 and H == _HQ and DH == _DH
    W = min(4096, max(256, SK // 4))

    kt = jnp.swapaxes(A_k_cache, 2, 3)
    vt = jnp.swapaxes(A_v_cache, 2, 3)
    x2 = A_x.reshape(1, D)

    wo_chunks = ((0, 8), (8, 13), (13, 15), (15, 16))
    bf16 = jnp.bfloat16
    any_spec = pl.BlockSpec(memory_space=pl.ANY)
    out = pl.pallas_call(
        _make_kernel(D, F, H, SK, W, wo_chunks),
        out_shape=jax.ShapeDtypeStruct((1, D), bf16),
        in_specs=[any_spec] * 8,
        out_specs=pl.BlockSpec(memory_space=pltpu.VMEM),
        scratch_shapes=[
            pltpu.VMEM((1, D), bf16),
            pltpu.VMEM((D, H * DH), bf16),
            pltpu.VMEM((H * DH, D), bf16),
            pltpu.VMEM((D, F), bf16),
            pltpu.VMEM((D, F), bf16),
            pltpu.VMEM((F, D), bf16),
            pltpu.VMEM((_NB, DH, W), bf16),
            pltpu.VMEM((_NB, DH, W), bf16),
            pltpu.VMEM((H, DH), jnp.float32),
            pltpu.VMEM((H, DH), jnp.float32),
            pltpu.SemaphoreType.DMA((5,)),
            pltpu.SemaphoreType.DMA((_NB,)),
            pltpu.SemaphoreType.DMA((_NB,)),
            pltpu.SemaphoreType.DMA((len(wo_chunks),)),
        ],
        compiler_params=pltpu.CompilerParams(vmem_limit_bytes=64 * 1024 * 1024),
    )(x2, kt, vt, A_wq, A_wo, B_w1, B_w3, B_w2)
    return out.reshape(B, Sq, D)
```

```python
import jax
import jax.numpy as jnp
from jax import lax
import jax.experimental.pallas as pl
import jax.experimental.pallas.tpu as pltpu

_HQ = 32
_DH = 192
_NB = 2
_EPS = 1e-5

_NN = (((1,), (0,)), ((), ()))
_NT = (((1,), (1,)), ((), ()))


def _silu(x):
    return x * jax.nn.sigmoid(x)


def _make_kernel(D, F, H, SK, W):
    DH = _DH
    NP = H // 2
    PW = 2 * DH
    scale = DH ** -0.5

    def kernel(x_hbm, kt_hbm, vt_hbm, wq_hbm, wo_hbm, w1_hbm, w3_hbm, w2_hbm,
               out_ref,
               x_v, wq_v, wo_v, w1_v, w3_v, w2_v, kbuf, vbuf, q_scr, o_scr,
               sem_w, sem_k, sem_v, sem_o):
        def k_copy(h, slot):
            return pltpu.make_async_copy(
                kt_hbm.at[0, h, :, pl.ds(SK - W, W)], kbuf.at[slot], sem_k.at[slot])

        def v_copy(h, slot):
            return pltpu.make_async_copy(
                vt_hbm.at[0, h, :, pl.ds(SK - W, W)], vbuf.at[slot], sem_v.at[slot])

        def wo_copy(h):
            r0 = pl.multiple_of(h * DH, DH)
            return pltpu.make_async_copy(
                wo_hbm.at[pl.ds(r0, DH), :], wo_v.at[pl.ds(r0, DH), :], sem_o.at[h])

        cx = pltpu.make_async_copy(x_hbm, x_v, sem_w.at[0])
        cq = pltpu.make_async_copy(wq_hbm, wq_v, sem_w.at[1])
        c1 = pltpu.make_async_copy(w1_hbm, w1_v, sem_w.at[2])
        c3 = pltpu.make_async_copy(w3_hbm, w3_v, sem_w.at[3])
        c2 = pltpu.make_async_copy(w2_hbm, w2_v, sem_w.at[4])

        cx.start()
        cq.start()
        c1.start()
        c3.start()
        c2.start()
        for s in range(_NB):
            k_copy(s, s).start()
            v_copy(s, s).start()

        def issue_wo(h, carry):
            wo_copy(h).start(priority=1)
            return carry

        lax.fori_loop(0, H, issue_wo, 0)

        cx.wait()
        x = x_v[...].astype(jnp.float32)
        mu = jnp.mean(x, axis=-1, keepdims=True)
        xc = x - mu
        var = jnp.mean(xc * xc, axis=-1, keepdims=True)
        xn = (xc / jnp.sqrt(var + _EPS)).astype(jnp.bfloat16)

        cq.wait()
        for p in range(NP):
            qp = lax.dot_general(xn, wq_v[:, p * PW:(p + 1) * PW], _NN,
                                 preferred_element_type=jnp.float32)
            q_scr[2 * p:2 * p + 1, :] = qp[:, :DH]
            q_scr[2 * p + 1:2 * p + 2, :] = qp[:, DH:]

        c1.wait()
        gate = lax.dot_general(xn, w1_v[...], _NN, preferred_element_type=jnp.float32)
        c3.wait()
        up = lax.dot_general(xn, w3_v[...], _NN, preferred_element_type=jnp.float32)
        hh = (_silu(gate) * up).astype(jnp.bfloat16)
        c2.wait()
        ffn = lax.dot_general(hh, w2_v[...], _NN, preferred_element_type=jnp.float32)
        g = _silu(ffn)

        def head(h, carry):
            slot = h % _NB
            q = q_scr[pl.ds(h, 1), :].astype(jnp.bfloat16)
            k_copy(h, slot).wait()
            s = lax.dot_general(q, kbuf[slot], _NN,
                                preferred_element_type=jnp.float32) * scale
            m = jnp.max(s, axis=-1, keepdims=True)
            p = jnp.exp(s - m)
            l = jnp.sum(p, axis=-1, keepdims=True)

            @pl.when(h + _NB < H)
            def _():
                k_copy(h + _NB, slot).start()

            v_copy(h, slot).wait()
            o = lax.dot_general(p.astype(jnp.bfloat16), vbuf[slot], _NT,
                                preferred_element_type=jnp.float32)
            o_scr[pl.ds(h, 1), :] = o / l

            @pl.when(h + _NB < H)
            def _():
                v_copy(h + _NB, slot).start()

            return carry

        lax.fori_loop(0, H, head, 0)

        def oproj(h, acc):
            oh = o_scr[pl.ds(h, 1), :].astype(jnp.bfloat16)
            wo_copy(h).wait()
            r0 = pl.multiple_of(h * DH, DH)
            return acc + lax.dot_general(
                oh, wo_v[pl.ds(r0, DH), :], _NN, preferred_element_type=jnp.float32)

        acc = lax.fori_loop(0, H, oproj, jnp.zeros((1, D), jnp.float32))

        out_ref[...] = (x + acc * g).astype(out_ref.dtype)

    return kernel


@jax.jit
def pallas_recurrent_scan__sliding_block_cached__glu_gated_swiglu__decode_kernel(
    A_x: jax.Array,
    A_k_cache: jax.Array,
    A_v_cache: jax.Array,
    A_wq: jax.Array,
    A_wo: jax.Array,
    B_x: jax.Array,
    B_w1: jax.Array,
    B_w3: jax.Array,
    B_w2: jax.Array,
):
    B, Sq, D = A_x.shape
    _, H, SK, DH = A_k_cache.shape
    F = B_w1.shape[1]
    assert B == 1 and Sq == 1 and H == _HQ and DH == _DH
    W = min(4096, max(256, SK // 4))

    kt = jnp.swapaxes(A_k_cache, 2, 3)
    vt = jnp.swapaxes(A_v_cache, 2, 3)
    x2 = A_x.reshape(1, D)

    bf16 = jnp.bfloat16
    any_spec = pl.BlockSpec(memory_space=pl.ANY)
    out = pl.pallas_call(
        _make_kernel(D, F, H, SK, W),
        out_shape=jax.ShapeDtypeStruct((1, D), bf16),
        in_specs=[any_spec] * 8,
        out_specs=pl.BlockSpec(memory_space=pltpu.VMEM),
        scratch_shapes=[
            pltpu.VMEM((1, D), bf16),
            pltpu.VMEM((D, H * DH), bf16),
            pltpu.VMEM((H * DH, D), bf16),
            pltpu.VMEM((D, F), bf16),
            pltpu.VMEM((D, F), bf16),
            pltpu.VMEM((F, D), bf16),
            pltpu.VMEM((_NB, DH, W), bf16),
            pltpu.VMEM((_NB, DH, W), bf16),
            pltpu.VMEM((H, DH), jnp.float32),
            pltpu.VMEM((H, DH), jnp.float32),
            pltpu.SemaphoreType.DMA((5,)),
            pltpu.SemaphoreType.DMA((_NB,)),
            pltpu.SemaphoreType.DMA((_NB,)),
            pltpu.SemaphoreType.DMA((H,)),
        ],
        compiler_params=pltpu.CompilerParams(
            vmem_limit_bytes=64 * 1024 * 1024,
            disable_bounds_checks=True,
            disable_semaphore_checks=True),
    )(x2, kt, vt, A_wq, A_wo, B_w1, B_w3, B_w2)
    return out.reshape(B, Sq, D)
```

```python
import jax
import jax.numpy as jnp
from jax import lax
import jax.experimental.pallas as pl
import jax.experimental.pallas.tpu as pltpu

_HQ = 32
_DH = 192
_EPS = 1e-5

_S = 8
_KV_SMALL = 384

_NN = (((1,), (0,)), ((), ()))
_NT = (((1,), (1,)), ((), ()))


def _silu(x):
    return x * jax.nn.sigmoid(x)


def _dot(a, b, dims=_NN):
    return lax.dot_general(a, b, dims, preferred_element_type=jnp.float32)


class _Step:
    def __init__(self, bulk, small):
        self.bulk, self.small = bulk, small

    def start(self):
        pltpu.make_async_copy(*self.bulk).start(priority=1)
        pltpu.make_async_copy(*self.small).start(priority=0)

    def wait_bulk(self):
        pltpu.make_async_copy(*self.bulk).wait()

    def wait_small(self):
        pltpu.make_async_copy(*self.small).wait()


def _col_step(src, dst, rows, csplit, cend, sem_bulk, sem_small, src_col0=0):
    return _Step(
        (src.at[rows, pl.ds(src_col0, csplit)], dst.at[rows, pl.ds(0, csplit)], sem_bulk),
        (src.at[rows, pl.ds(src_col0 + csplit, cend - csplit)],
         dst.at[rows, pl.ds(csplit, cend - csplit)], sem_small))


def _wait_region(ref, sem):
    pltpu.make_async_copy(ref, ref, sem).wait()


def _make_kernel(D, F, H, SK, W):
    DH = _DH
    S = _S
    NP = H // 2
    PW = 2 * DH
    CW = W // S
    GR = DH // S
    C1 = W - _KV_SMALL
    scale = DH ** -0.5

    WQ_R, WQ_C1 = 16, H * DH - 512
    W1_R, W1_C1 = 64, F - 128
    W2_N = 8
    W2_SMALL = 16
    W2_BULK = F // W2_N - W2_SMALL
    WO_SMALL = 16

    def kernel(x_hbm, kt_hbm, vt_hbm, wq_hbm, wo_hbm, w1_hbm, w3_hbm, w2_hbm,
               out_ref,
               x_v, wq_v, wo_v, w1_v, w3_v, w2_v, kbuf, vbuf, q_scr, o_scr,
               sem_x, sem_wb, sem_ws, sem_kb, sem_ks, sem_vb, sem_vs, sem_o):

        def kv_step(hbm, buf, sem_b, sem_s, h, slot, i):
            return _col_step(hbm.at[0, h], buf.at[slot], pl.ds(i * GR, GR), C1, W,
                             sem_b.at[slot], sem_s.at[slot], src_col0=SK - W)

        def k_step(h, slot, i):
            return kv_step(kt_hbm, kbuf, sem_kb, sem_ks, h, slot, i)

        def v_step(h, slot, i):
            return kv_step(vt_hbm, vbuf, sem_vb, sem_vs, h, slot, i)

        def wo_step(g):
            r0 = g * DH
            if not isinstance(g, int):
                r0 = pl.multiple_of(r0, DH)
            nb = DH - WO_SMALL
            r1 = r0 + nb
            if not isinstance(g, int):
                r1 = pl.multiple_of(r1, WO_SMALL)
            rb, rs = pl.ds(r0, nb), pl.ds(r1, WO_SMALL)
            return _Step((wo_hbm.at[rb, :], wo_v.at[rb, :], sem_o.at[g]),
                         (wo_hbm.at[rs, :], wo_v.at[rs, :], sem_o.at[g]))

        steps = []
        for t in range(D // WQ_R):
            steps.append(_col_step(wq_hbm, wq_v, pl.ds(t * WQ_R, WQ_R), WQ_C1, H * DH,
                                   sem_wb.at[0], sem_ws.at[0]))
        t_w1 = len(steps)
        for t in range(D // W1_R):
            steps.append(_col_step(w1_hbm, w1_v, pl.ds(t * W1_R, W1_R), W1_C1, F,
                                   sem_wb.at[1], sem_ws.at[1]))
        t_w3 = len(steps)
        for t in range(D // W1_R):
            steps.append(_col_step(w3_hbm, w3_v, pl.ds(t * W1_R, W1_R), W1_C1, F,
                                   sem_wb.at[2], sem_ws.at[2]))
        t_w2 = len(steps)
        for t in range(W2_N):
            rb = pl.ds(t * W2_BULK, W2_BULK)
            rs = pl.ds(W2_N * W2_BULK + t * W2_SMALL, W2_SMALL)
            steps.append(_Step((w2_hbm.at[rb, :], w2_v.at[rb, :], sem_wb.at[3]),
                               (w2_hbm.at[rs, :], w2_v.at[rs, :], sem_ws.at[3])))
        t_k0 = len(steps)
        for i in range(S):
            steps.append(k_step(0, 0, i))
        n_a = len(steps)
        for i in range(S):
            steps.append(v_step(0, 0, i))

        cx = pltpu.make_async_copy(x_hbm, x_v, sem_x.at[0])
        cx.start()
        for t in range(S):
            steps[t].start()

        vals = {}

        def do_ln():
            cx.wait()
            x = x_v[...].astype(jnp.float32)
            mu = jnp.mean(x, axis=-1, keepdims=True)
            xc = x - mu
            var = jnp.mean(xc * xc, axis=-1, keepdims=True)
            vals["x"] = x
            vals["xn"] = (xc / jnp.sqrt(var + _EPS)).astype(jnp.bfloat16)

        def do_q(p):
            if p == 0:
                _wait_region(wq_v.at[:, pl.ds(WQ_C1, H * DH - WQ_C1)], sem_ws.at[0])
            qp = _dot(vals["xn"], wq_v[:, p * PW:(p + 1) * PW])
            q_scr[2 * p:2 * p + 1, :] = qp[:, :DH]
            q_scr[2 * p + 1:2 * p + 2, :] = qp[:, DH:]

        NFC = F // PW

        def do_gate(c):
            if c == 0:
                _wait_region(w1_v.at[:, pl.ds(W1_C1, F - W1_C1)], sem_ws.at[1])
            vals["gate", c] = _dot(vals["xn"], w1_v[:, c * PW:(c + 1) * PW])

        def do_up(c):
            if c == 0:
                _wait_region(w3_v.at[:, pl.ds(W1_C1, F - W1_C1)], sem_ws.at[2])
            up = _dot(vals["xn"], w3_v[:, c * PW:(c + 1) * PW])
            vals["hh", c] = (_silu(vals["gate", c]) * up).astype(jnp.bfloat16)

        def do_ffn(c):
            if c == 0:
                _wait_region(w2_v.at[pl.ds(W2_N * W2_BULK, W2_N * W2_SMALL), :], sem_ws.at[3])
            part = _dot(vals["hh", c], w2_v[c * PW:(c + 1) * PW, :])
            vals["ffn"] = part if c == 0 else vals["ffn"] + part

        work = {t: [] for t in range(n_a)}
        work[0].append(do_ln)
        for p in range(NP):
            work[t_w1 + p].append(lambda p=p: do_q(p))
        for c in range(NFC):
            work[t_w1 + NP + c].append(lambda c=c: do_gate(c))
        for c in range(NFC):
            work[max(t_w2, t_w1 + NP + NFC) + c].append(lambda c=c: do_up(c))
        for c in range(NFC):
            work[t_k0 + 2 * c].append(lambda c=c: do_ffn(c))
        assert t_w1 + NP >= t_w3

        for t in range(n_a):
            steps[t].wait_bulk()
            steps[t + S].start()
            for fn in work[t]:
                fn()

        x = vals["x"]
        g = _silu(vals["ffn"])

        row = lax.broadcasted_iota(jnp.int32, (8, 1), 0)

        def head(h, slot, last):
            nslot = 1 - slot
            q = q_scr[pl.ds(h, 1), :].astype(jnp.bfloat16)
            q8 = jnp.broadcast_to(q, (S, DH))
            _wait_region(kbuf.at[slot, :, pl.ds(C1, W - C1)], sem_ks.at[slot])
            s_all = jnp.zeros((S, CW), jnp.float32)
            for i in range(S):
                v_step(h, slot, i).wait_bulk()
                (wo_step(i) if last else k_step(h + 1, nslot, i)).start()
                res = _dot(q8, kbuf[slot, :, i * CW:(i + 1) * CW])
                s_all = jnp.where(row == i, res, s_all)
            s_all = s_all * scale
            m = jnp.max(jnp.max(s_all, axis=1, keepdims=True), axis=0, keepdims=True)
            p = jnp.exp(s_all - m)
            l = jnp.sum(jnp.sum(p, axis=1, keepdims=True), axis=0, keepdims=True)
            pb = p.astype(jnp.bfloat16)
            _wait_region(vbuf.at[slot, :, pl.ds(C1, W - C1)], sem_vs.at[slot])
            acc = jnp.zeros((S, DH), jnp.float32)
            for i in range(S):
                if last:
                    wo_step(i).wait_bulk()
                    wo_step(S + i).start()
                else:
                    k_step(h + 1, nslot, i).wait_bulk()
                    v_step(h + 1, nslot, i).start()
                res = _dot(pb, vbuf[slot, :, i * CW:(i + 1) * CW], _NT)
                acc = acc + jnp.where(row == i, res, 0.0)
            o_scr[pl.ds(h, 1), :] = jnp.sum(acc, axis=0, keepdims=True) / l

        def head_loop(h, carry):
            head(h, h % 2, False)
            return carry

        lax.fori_loop(0, H - 1, head_loop, 0)
        head(H - 1, (H - 1) % 2, True)

        def oproj(gi, acc):
            oh = o_scr[pl.ds(gi, 1), :].astype(jnp.bfloat16)

            @pl.when(gi >= S)
            def _():
                wo_step(gi).wait_bulk()

            @pl.when(jnp.logical_and(gi >= S, gi + S < H))
            def _():
                wo_step(gi + S).start()

            wo_step(gi).wait_small()
            r0 = pl.multiple_of(gi * DH, DH)
            return acc + _dot(oh, wo_v[pl.ds(r0, DH), :])

        acc = lax.fori_loop(0, H, oproj, jnp.zeros((1, D), jnp.float32))

        out_ref[...] = (x + acc * g).astype(out_ref.dtype)

    return kernel


@jax.jit
def pallas_recurrent_scan__sliding_block_cached__glu_gated_swiglu__decode_kernel(
    A_x: jax.Array,
    A_k_cache: jax.Array,
    A_v_cache: jax.Array,
    A_wq: jax.Array,
    A_wo: jax.Array,
    B_x: jax.Array,
    B_w1: jax.Array,
    B_w3: jax.Array,
    B_w2: jax.Array,
):
    B, Sq, D = A_x.shape
    _, H, SK, DH = A_k_cache.shape
    F = B_w1.shape[1]
    assert B == 1 and Sq == 1 and H == _HQ and DH == _DH
    W = min(4096, max(256, SK // 4))

    kt = jnp.swapaxes(A_k_cache, 2, 3)
    vt = jnp.swapaxes(A_v_cache, 2, 3)
    x2 = A_x.reshape(1, D)

    bf16 = jnp.bfloat16
    dma = pltpu.SemaphoreType.DMA
    any_spec = pl.BlockSpec(memory_space=pl.ANY)
    out = pl.pallas_call(
        _make_kernel(D, F, H, SK, W),
        out_shape=jax.ShapeDtypeStruct((1, D), bf16),
        in_specs=[any_spec] * 8,
        out_specs=pl.BlockSpec(memory_space=pltpu.VMEM),
        scratch_shapes=[
            pltpu.VMEM((1, D), bf16),
            pltpu.VMEM((D, H * DH), bf16),
            pltpu.VMEM((H * DH, D), bf16),
            pltpu.VMEM((D, F), bf16),
            pltpu.VMEM((D, F), bf16),
            pltpu.VMEM((F, D), bf16),
            pltpu.VMEM((2, DH, W), bf16),
            pltpu.VMEM((2, DH, W), bf16),
            pltpu.VMEM((H, DH), jnp.float32),
            pltpu.VMEM((H, DH), jnp.float32),
            dma((1,)), dma((4,)), dma((4,)),
            dma((2,)), dma((2,)), dma((2,)), dma((2,)),
            dma((H,)),
        ],
        compiler_params=pltpu.CompilerParams(
            vmem_limit_bytes=64 * 1024 * 1024,
            disable_bounds_checks=True,
            disable_semaphore_checks=True),
    )(x2, kt, vt, A_wq, A_wo, B_w1, B_w3, B_w2)
    return out.reshape(B, Sq, D)
```

```python
import jax
import jax.numpy as jnp
from jax import lax
import jax.experimental.pallas as pl
import jax.experimental.pallas.tpu as pltpu

_HQ = 32
_DH = 192
_EPS = 1e-5

_LA = 16
_RC = 48
_CC = 1024
_CW = 512
_SM = 8

_NN = (((1,), (0,)), ((), ()))
_NT = (((1,), (1,)), ((), ()))


def _silu(x):
    return x * jax.nn.sigmoid(x)


def _dot(a, b, dims=_NN):
    return lax.dot_general(a, b, dims, preferred_element_type=jnp.float32)


def _copy(src, dst, sem):
    return pltpu.make_async_copy(src, dst, sem)


def _wait_region(ref, sem):
    pltpu.make_async_copy(ref, ref, sem).wait()


def _make_kernel(D, F, H, SK, W):
    DH = _DH
    LA = _LA
    NR = DH // _RC
    NC = W // _CC
    NCH = W // _CW
    PW = 2 * DH
    scale = DH ** -0.5
    assert NR * NC == LA and NCH == 8

    A = 4
    W1_R = 8
    W2_R = 16
    WQ_R = 16
    NQ = D // 2 // WQ_R
    WO_R = 16
    NO = DH // WO_R
    ROT = 5

    def kernel(x_hbm, kt_hbm, vt_hbm, wq_hbm, wo_hbm, w1_hbm, w3_hbm, w2_hbm,
               out_ref,
               x_v, wq_v, wo_v, w1_v, w3_v, w2_v, kbuf, vbuf, q_scr,
               sem_x, sem_w, sem_q, sem_o, sem_k, sem_ks, sem_v, sem_vs):

        def is_split(kind, h, k):
            if not isinstance(h, int):
                return False
            if h < H - 2:
                return False
            if h == H - 2:
                return kind == "v" and k >= ROT
            return True

        def kv_copy(kind, h, k, part):
            hbm, buf = (kt_hbm, kbuf) if kind == "k" else (vt_hbm, vbuf)
            c, r = divmod(k, NR)
            if part == "full":
                rows, sem = pl.ds(r * _RC, _RC), (sem_k if kind == "k" else sem_v)
            elif part == "bulk":
                rows, sem = pl.ds(r * _RC, _RC - _SM), (sem_k if kind == "k" else sem_v)
            else:
                rows, sem = pl.ds(r * _RC + _RC - _SM, _SM), (sem_ks if kind == "k" else sem_vs)
            return _copy(hbm.at[0, h, rows, pl.ds(SK - W + c * _CC, _CC)],
                         buf.at[rows, pl.ds(c * _CC, _CC)], sem.at[c])

        def kv_start(kind, h, k):
            if is_split(kind, h, k):
                kv_copy(kind, h, k, "bulk").start(priority=1)
                kv_copy(kind, h, k, "small").start(priority=0)
            else:
                kv_copy(kind, h, k, "full").start(priority=1)

        def kv_wait(kind, h, k):
            kv_copy(kind, h, k, "bulk" if is_split(kind, h, k) else "full").wait()

        def kv_wait_small(kind, h, c):
            for k in range(c * NR, (c + 1) * NR):
                if is_split(kind, h, k):
                    kv_copy(kind, h, k, "small").wait()

        def wq_copy(p, r0, n):
            if not isinstance(r0, int):
                r0 = pl.multiple_of(r0, 8)
            c0 = p * PW
            if not isinstance(c0, int):
                c0 = pl.multiple_of(c0, 128)
            return _copy(wq_hbm.at[pl.ds(r0, n), pl.ds(c0, PW)], wq_v.at[p, pl.ds(r0, n), :], sem_q.at[0])

        def wo_copy(h, j, n):
            r0 = h * DH + j * n
            if not isinstance(r0, int):
                r0 = pl.multiple_of(r0, 8)
            return _copy(wo_hbm.at[pl.ds(r0, n), :], wo_v.at[h, pl.ds(j * n, n), :], sem_o.at[0])

        a_steps = []
        for j in range(D // A // W1_R):
            rows = pl.ds(j * W1_R, W1_R)
            a_steps.append(_copy(w1_hbm.at[:, rows, :], w1_v.at[:, rows, :], sem_w.at[0]))
        t_w3 = len(a_steps)
        for j in range(D // A // W1_R):
            rows = pl.ds(j * W1_R, W1_R)
            a_steps.append(_copy(w3_hbm.at[:, rows, :], w3_v.at[:, rows, :], sem_w.at[1]))
        t_w2 = len(a_steps)
        for j in range(F // A // W2_R):
            rows = pl.ds(j * W2_R, W2_R)
            a_steps.append(_copy(w2_hbm.at[:, rows, :], w2_v.at[:, rows, :], sem_w.at[2]))
        n_a = len(a_steps)

        a_small = [wq_copy(0, j * WQ_R, WQ_R) for j in range(D // WQ_R)]
        t_wo0 = len(a_small)
        a_small += [wo_copy(0, j, 8) for j in range(DH // 8)]
        assert len(a_small) == n_a

        cx = _copy(x_hbm, x_v, sem_x.at[0])
        cx.start()
        for t in range(LA):
            a_steps[t].start(priority=1)

        vals = {}

        def do_ln():
            cx.wait()
            x = x_v[...].astype(jnp.float32)
            mu = jnp.mean(x, axis=-1, keepdims=True)
            xc = x - mu
            var = jnp.mean(xc * xc, axis=-1, keepdims=True)
            vals["x"] = x
            vals["xn"] = (xc / jnp.sqrt(var + _EPS)).astype(jnp.bfloat16)

        def do_q(p):
            _wait_region(wq_v.at[p], sem_q.at[0])
            qp = _dot(vals["xn"], wq_v[p])
            q_scr[pl.ds(2 * p, 1), :] = qp[:, :DH]
            q_scr[pl.ds(2 * p + 1, 1), :] = qp[:, DH:]

        NFC = F // PW

        def do_gate(c):
            w = w1_v[:, :, c * PW:(c + 1) * PW].reshape(D, PW)
            vals["gate", c] = _dot(vals["xn"], w)

        def do_up(c):
            w = w3_v[:, :, c * PW:(c + 1) * PW].reshape(D, PW)
            up = _dot(vals["xn"], w)
            vals["hh", c] = (_silu(vals["gate", c]) * up).astype(jnp.bfloat16)

        def do_ffn(a):
            hh = jnp.concatenate([vals["hh", c] for c in range(NFC)], axis=1) if "hh" not in vals else vals["hh"]
            vals["hh"] = hh
            rows = F // A
            part = _dot(hh[:, a * rows:(a + 1) * rows], w2_v[a])
            vals["ffn"] = part if a == 0 else vals["ffn"] + part

        work = {t: [] for t in range(n_a + ROT)}
        work[0].append(do_ln)
        for c in range(NFC):
            work[t_w3 + c].append(lambda c=c: do_gate(c))
        for c in range(NFC):
            work[t_w2 + c].append(lambda c=c: do_up(c))
        work[t_wo0 + 6].append(lambda: do_q(0))
        for a in range(A):
            work[n_a + a].append(lambda a=a: do_ffn(a))

        for t in range(n_a):
            a_steps[t].wait()
            if t + LA < n_a:
                a_steps[t + LA].start(priority=1)
            else:
                kv_start("k", 0, t + LA - n_a)
            a_small[t].start(priority=0)
            for fn in work[t]:
                fn()
        for k in range(ROT):
            kv_wait("k", 0, k)
            kv_start("v", 0, k)
            for fn in work[n_a + k]:
                fn()

        x = vals["x"]
        xn = vals["xn"]
        g = _silu(vals["ffn"])

        row = lax.broadcasted_iota(jnp.int32, (8, 1), 0)

        def head(h, acc):
            static = isinstance(h, int)
            last = static and h == H - 1
            st = {}

            def qk(j):
                def f():
                    if j % 2 == 0:
                        kv_wait_small("k", h, j // 2)
                    if j == 0:
                        q = q_scr[pl.ds(h, 1), :].astype(jnp.bfloat16)
                        st["q8"] = jnp.broadcast_to(q, (8, DH))
                        st["s"] = jnp.zeros((8, _CW), jnp.float32)
                    res = _dot(st["q8"], kbuf[:, j * _CW:(j + 1) * _CW])
                    st["s"] = jnp.where(row == j, res, st["s"])
                return f

            def smax():
                s = st["s"] * scale
                st["s"] = s
                st["m"] = jnp.max(jnp.max(s, axis=1, keepdims=True), axis=0, keepdims=True)

            def sexp():
                p = jnp.exp(st["s"] - st["m"])
                st["l"] = jnp.sum(jnp.sum(p, axis=1, keepdims=True), axis=0, keepdims=True)
                st["pb"] = p.astype(jnp.bfloat16)
                st["o"] = jnp.zeros((8, DH), jnp.float32)

            def pv(j):
                def f():
                    if j % 2 == 0:
                        kv_wait_small("v", h, j // 2)
                    res = _dot(st["pb"], vbuf[:, j * _CW:(j + 1) * _CW], _NT)
                    st["o"] = st["o"] + jnp.where(row == j, res, 0.0)
                return f

            def fin():
                o = jnp.sum(st["o"], axis=0, keepdims=True) / st["l"]
                st["ob"] = o.astype(jnp.bfloat16)

            def wo_wait():
                _wait_region(wo_v.at[h], sem_o.at[0])

            def oproj():
                st["acc"] = acc + _dot(st["ob"], wo_v[h])

            def qproj():
                if static:
                    return
                @pl.when(h % 2 == 1)
                def _():
                    p = (h + 1) // 2
                    _wait_region(wq_v.at[p], sem_q.at[0])
                    qp = _dot(xn, wq_v[p])
                    q_scr[pl.ds(2 * p, 1), :] = qp[:, :DH]
                    q_scr[pl.ds(2 * p + 1, 1), :] = qp[:, DH:]

            comp = {0: qk(0), 1: qk(1), 3: qk(2), 5: qk(3), 7: qk(4), 9: qk(5), 10: qk(6), 11: qk(7),
                    12: smax, 13: sexp,
                    14: pv(0), 16: pv(1), 18: pv(2), 20: pv(3), 22: pv(4), 24: pv(5), 26: pv(6), 27: pv(7),
                    28: fin, 4: wo_wait, 30: oproj, 25: qproj}

            seq = ([("k", h, k) for k in range(ROT, LA)] + [("v", h, k) for k in range(LA)]
                   + [("k", h + 1, k) for k in range(ROT)])
            for sg, (kind, hh, k) in enumerate(seq):
                if last and sg >= 27:
                    break
                kv_wait(kind, hh, k)
                if kind == "k":
                    kv_start("v", hh, k)
                elif not last:
                    kv_start("k", h + 1, k)
                elif k == 0:
                    _copy(wo_hbm.at[pl.ds(h * DH, DH), :], wo_v.at[h], sem_o.at[0]).start(priority=1)
                if not static:
                    if sg < NQ:
                        wq_copy((h + 2) // 2, (h % 2) * (D // 2) + sg * WQ_R, WQ_R).start(priority=0)
                    else:
                        wo_copy(h + 1, sg - NQ, WO_R).start(priority=0)
                if last and sg == 4:
                    continue
                if sg in comp:
                    comp[sg]()
            if last:
                pv(7)()
                fin()
                wo_wait()
                oproj()
            return st["acc"]

        acc = lax.fori_loop(0, H - 2, head, jnp.zeros((1, D), jnp.float32))
        acc = head(H - 2, acc)
        acc = head(H - 1, acc)

        out_ref[...] = (x + acc * g).astype(out_ref.dtype)

    return kernel


@jax.jit
def pallas_recurrent_scan__sliding_block_cached__glu_gated_swiglu__decode_kernel(
    A_x: jax.Array,
    A_k_cache: jax.Array,
    A_v_cache: jax.Array,
    A_wq: jax.Array,
    A_wo: jax.Array,
    B_x: jax.Array,
    B_w1: jax.Array,
    B_w3: jax.Array,
    B_w2: jax.Array,
):
    B, Sq, D = A_x.shape
    _, H, SK, DH = A_k_cache.shape
    F = B_w1.shape[1]
    assert B == 1 and Sq == 1 and H == _HQ and DH == _DH
    W = min(4096, max(256, SK // 4))

    kt = jnp.swapaxes(A_k_cache, 2, 3)
    vt = jnp.swapaxes(A_v_cache, 2, 3)
    x2 = A_x.reshape(1, D)
    w1 = B_w1.reshape(4, D // 4, F)
    w3 = B_w3.reshape(4, D // 4, F)
    w2 = B_w2.reshape(4, F // 4, D)

    bf16 = jnp.bfloat16
    dma = pltpu.SemaphoreType.DMA
    any_spec = pl.BlockSpec(memory_space=pl.ANY)
    out = pl.pallas_call(
        _make_kernel(D, F, H, SK, W),
        out_shape=jax.ShapeDtypeStruct((1, D), bf16),
        in_specs=[any_spec] * 8,
        out_specs=pl.BlockSpec(memory_space=pltpu.VMEM),
        scratch_shapes=[
            pltpu.VMEM((1, D), bf16),
            pltpu.VMEM((H // 2, D, 2 * DH), bf16),
            pltpu.VMEM((H, DH, D), bf16),
            pltpu.VMEM((4, D // 4, F), bf16),
            pltpu.VMEM((4, D // 4, F), bf16),
            pltpu.VMEM((4, F // 4, D), bf16),
            pltpu.VMEM((DH, W), bf16),
            pltpu.VMEM((DH, W), bf16),
            pltpu.VMEM((H, DH), jnp.float32),
            dma((1,)), dma((3,)), dma((1,)), dma((1,)),
            dma((4,)), dma((4,)), dma((4,)), dma((4,)),
        ],
        compiler_params=pltpu.CompilerParams(
            vmem_limit_bytes=64 * 1024 * 1024,
            disable_bounds_checks=True,
            disable_semaphore_checks=True),
    )(x2, kt, vt, A_wq, A_wo, w1, w3, w2)
    return out.reshape(B, Sq, D)
```

```python
import jax
import jax.numpy as jnp
from jax import lax
import jax.experimental.pallas as pl
import jax.experimental.pallas.tpu as pltpu

_HQ = 32
_DH = 192
_EPS = 1e-5

_RC = 24
_LA = 24
_LA_A = 16
_CC = 1024
_CW = 512
_SM = 8

_WQ_R = 8
_WO_R = 8
_ROT = 8
_QK_AT = (0, 4, 8, 12, 16, 20, 23, 26)
_SMAX_AT, _SEXP_AT = 28, 29
_PV_AT = (32, 36, 40, 44, 48, 52, 55, 58)
_FIN_AT, _OPROJ_AT, _WOWAIT_AT, _QPROJ_AT = 60, 62, 30, 46

_NN = (((1,), (0,)), ((), ()))
_NT = (((1,), (1,)), ((), ()))


def _silu(x):
    return x * jax.nn.sigmoid(x)


def _dot(a, b, dims=_NN):
    return lax.dot_general(a, b, dims, preferred_element_type=jnp.float32)


def _copy(src, dst, sem):
    return pltpu.make_async_copy(src, dst, sem)


def _wait_region(ref, sem):
    pltpu.make_async_copy(ref, ref, sem).wait()


def _make_kernel(D, F, H, SK, W):
    DH = _DH
    LA = _LA
    NR = DH // _RC
    NC = W // _CC
    NCH = W // _CW
    PW = 2 * DH
    scale = DH ** -0.5
    NPC = NR * NC
    assert LA <= NPC and NCH == 8

    A = 4
    W1_R = 8
    W2_R = 16
    WQ_R = _WQ_R
    NQ = D // 2 // WQ_R
    WO_R = _WO_R
    NO = DH // WO_R
    ROT = _ROT
    assert NQ + NO <= 2 * NPC

    def kernel(x_hbm, kt_hbm, vt_hbm, wq_hbm, wo_hbm, w1_hbm, w3_hbm, w2_hbm,
               out_ref,
               x_v, wq_v, wo_v, w1_v, w3_v, w2_v, kbuf, vbuf, q_scr,
               sem_x, sem_w, sem_q, sem_o, sem_k, sem_ks, sem_v, sem_vs):

        def is_split(kind, h, k):
            if not isinstance(h, int):
                return False
            if h < H - 2:
                return False
            if h == H - 2:
                return kind == "v" and k + NPC - LA >= ROT
            return True

        def kv_copy(kind, h, k, part):
            hbm, buf = (kt_hbm, kbuf) if kind == "k" else (vt_hbm, vbuf)
            c, r = divmod(k, NR)
            if part == "full":
                rows, sem = pl.ds(r * _RC, _RC), (sem_k if kind == "k" else sem_v)
            elif part == "bulk":
                rows, sem = pl.ds(r * _RC, _RC - _SM), (sem_k if kind == "k" else sem_v)
            else:
                rows, sem = pl.ds(r * _RC + _RC - _SM, _SM), (sem_ks if kind == "k" else sem_vs)
            return _copy(hbm.at[0, h, rows, pl.ds(SK - W + c * _CC, _CC)],
                         buf.at[rows, pl.ds(c * _CC, _CC)], sem.at[c])

        def kv_start(kind, h, k):
            if is_split(kind, h, k):
                kv_copy(kind, h, k, "bulk").start(priority=1)
                kv_copy(kind, h, k, "small").start(priority=0)
            else:
                kv_copy(kind, h, k, "full").start(priority=1)

        def kv_wait(kind, h, k):
            kv_copy(kind, h, k, "bulk" if is_split(kind, h, k) else "full").wait()

        def kv_wait_small(kind, h, c):
            for k in range(c * NR, (c + 1) * NR):
                if is_split(kind, h, k):
                    kv_copy(kind, h, k, "small").wait()

        def kv_ahead(kind, h, k):
            k2 = k + LA
            if k2 < NPC:
                return kind, h, k2
            if kind == "k":
                return "v", h, k2 - NPC
            return "k", h + 1, k2 - NPC

        def wq_copy(p, r0, n):
            if not isinstance(r0, int):
                r0 = pl.multiple_of(r0, 8)
            c0 = p * PW
            if not isinstance(c0, int):
                c0 = pl.multiple_of(c0, 128)
            return _copy(wq_hbm.at[pl.ds(r0, n), pl.ds(c0, PW)], wq_v.at[p, pl.ds(r0, n), :], sem_q.at[0])

        def wo_copy(h, j, n):
            r0 = h * DH + j * n
            if not isinstance(r0, int):
                r0 = pl.multiple_of(r0, 8)
            return _copy(wo_hbm.at[pl.ds(r0, n), :], wo_v.at[h, pl.ds(j * n, n), :], sem_o.at[0])

        a_steps = []
        for j in range(D // A // W1_R):
            rows = pl.ds(j * W1_R, W1_R)
            a_steps.append(_copy(w1_hbm.at[:, rows, :], w1_v.at[:, rows, :], sem_w.at[0]))
        t_w3 = len(a_steps)
        for j in range(D // A // W1_R):
            rows = pl.ds(j * W1_R, W1_R)
            a_steps.append(_copy(w3_hbm.at[:, rows, :], w3_v.at[:, rows, :], sem_w.at[1]))
        t_w2 = len(a_steps)
        for j in range(F // A // W2_R):
            rows = pl.ds(j * W2_R, W2_R)
            a_steps.append(_copy(w2_hbm.at[:, rows, :], w2_v.at[:, rows, :], sem_w.at[2]))
        n_a = len(a_steps)

        a_small = [wq_copy(0, j * 16, 16) for j in range(D // 16)]
        t_wo0 = len(a_small)
        a_small += [wo_copy(0, j, 8) for j in range(DH // 8)]
        assert len(a_small) == n_a

        cx = _copy(x_hbm, x_v, sem_x.at[0])
        cx.start()
        for t in range(_LA_A):
            a_steps[t].start(priority=1)

        vals = {}

        def do_ln():
            cx.wait()
            x = x_v[...].astype(jnp.float32)
            mu = jnp.mean(x, axis=-1, keepdims=True)
            xc = x - mu
            var = jnp.mean(xc * xc, axis=-1, keepdims=True)
            vals["x"] = x
            vals["xn"] = (xc / jnp.sqrt(var + _EPS)).astype(jnp.bfloat16)

        def do_q(p):
            _wait_region(wq_v.at[p], sem_q.at[0])
            qp = _dot(vals["xn"], wq_v[p])
            q_scr[pl.ds(2 * p, 1), :] = qp[:, :DH]
            q_scr[pl.ds(2 * p + 1, 1), :] = qp[:, DH:]

        NFC = F // PW

        def do_gate(c):
            w = w1_v[:, :, c * PW:(c + 1) * PW].reshape(D, PW)
            vals["gate", c] = _dot(vals["xn"], w)

        def do_up(c):
            w = w3_v[:, :, c * PW:(c + 1) * PW].reshape(D, PW)
            up = _dot(vals["xn"], w)
            vals["hh", c] = (_silu(vals["gate", c]) * up).astype(jnp.bfloat16)

        def do_ffn(a):
            hh = jnp.concatenate([vals["hh", c] for c in range(NFC)], axis=1) if "hh" not in vals else vals["hh"]
            vals["hh"] = hh
            rows = F // A
            part = _dot(hh[:, a * rows:(a + 1) * rows], w2_v[a])
            vals["ffn"] = part if a == 0 else vals["ffn"] + part

        work = {t: [] for t in range(n_a + ROT)}
        work[0].append(do_ln)
        for c in range(NFC):
            work[t_w3 + c].append(lambda c=c: do_gate(c))
        for c in range(NFC):
            work[t_w2 + c].append(lambda c=c: do_up(c))
        work[t_wo0 + 6].append(lambda: do_q(0))
        for a in range(A):
            work[n_a + (a * ROT) // A].append(lambda a=a: do_ffn(a))

        k0_at = {t: [] for t in range(n_a)}
        for k in range(LA):
            k0_at[n_a - _LA_A + (k * _LA_A) // LA].append(k)
        for t in range(n_a):
            a_steps[t].wait()
            if t + _LA_A < n_a:
                a_steps[t + _LA_A].start(priority=1)
            for k in k0_at[t]:
                kv_start("k", 0, k)
            a_small[t].start(priority=0)
            for fn in work[t]:
                fn()
        for k in range(ROT):
            kv_wait("k", 0, k)
            kv_start(*kv_ahead("k", 0, k))
            for fn in work[n_a + k]:
                fn()

        x = vals["x"]
        xn = vals["xn"]
        g = _silu(vals["ffn"])

        row = lax.broadcasted_iota(jnp.int32, (8, 1), 0)

        def head(h, acc):
            static = isinstance(h, int)
            last = static and h == H - 1
            st = {}

            def qk(j):
                def f():
                    if j % 2 == 0:
                        kv_wait_small("k", h, j // 2)
                    if j == 0:
                        q = q_scr[pl.ds(h, 1), :].astype(jnp.bfloat16)
                        st["q8"] = jnp.broadcast_to(q, (8, DH))
                        st["s"] = jnp.zeros((8, _CW), jnp.float32)
                    res = _dot(st["q8"], kbuf[:, j * _CW:(j + 1) * _CW])
                    st["s"] = jnp.where(row == j, res, st["s"])
                return f

            def smax():
                s = st["s"] * scale
                st["s"] = s
                st["m"] = jnp.max(jnp.max(s, axis=1, keepdims=True), axis=0, keepdims=True)

            def sexp():
                p = jnp.exp(st["s"] - st["m"])
                st["l"] = jnp.sum(jnp.sum(p, axis=1, keepdims=True), axis=0, keepdims=True)
                st["pb"] = p.astype(jnp.bfloat16)
                st["o"] = jnp.zeros((8, DH), jnp.float32)

            def pv(j):
                def f():
                    if j % 2 == 0:
                        kv_wait_small("v", h, j // 2)
                    res = _dot(st["pb"], vbuf[:, j * _CW:(j + 1) * _CW], _NT)
                    st["o"] = st["o"] + jnp.where(row == j, res, 0.0)
                return f

            def fin():
                o = jnp.sum(st["o"], axis=0, keepdims=True) / st["l"]
                st["ob"] = o.astype(jnp.bfloat16)

            def wo_wait():
                _wait_region(wo_v.at[h], sem_o.at[0])

            def oproj():
                st["acc"] = acc + _dot(st["ob"], wo_v[h])

            def qproj():
                if static:
                    return
                @pl.when(h % 2 == 1)
                def _():
                    p = (h + 1) // 2
                    _wait_region(wq_v.at[p], sem_q.at[0])
                    qp = _dot(xn, wq_v[p])
                    q_scr[pl.ds(2 * p, 1), :] = qp[:, :DH]
                    q_scr[pl.ds(2 * p + 1, 1), :] = qp[:, DH:]

            def both(*fns):
                def f():
                    for fn in fns:
                        fn()
                return f

            nk_steps = NPC - ROT
            if not last:
                items = [(_WOWAIT_AT, wo_wait)]
                items += [(_QK_AT[j], qk(j)) for j in range(NCH)]
                items += [(_SMAX_AT, smax), (_SEXP_AT, sexp)]
                items += [(_PV_AT[j], pv(j)) for j in range(NCH)]
                items += [(_FIN_AT, fin), (_OPROJ_AT, oproj), (_QPROJ_AT, qproj)]
                comp = {}
                for pos, fn in items:
                    comp[pos] = both(comp[pos], fn) if pos in comp else fn
            else:
                comp = {}
                for j in range(NCH - 2):
                    pos = _QK_AT[j]
                    comp[pos] = both(comp[pos], qk(j)) if pos in comp else qk(j)
                comp[nk_steps - 1] = both(qk(NCH - 2), qk(NCH - 1))
                comp[nk_steps] = both(smax, sexp)
                for c in range(NC):
                    comp[nk_steps + (c + 1) * NR - 1] = both(pv(2 * c), pv(2 * c + 1))

            seq = ([("k", h, k) for k in range(ROT, NPC)] + [("v", h, k) for k in range(NPC)]
                   + [("k", h + 1, k) for k in range(ROT)])
            n_last = 2 * NPC - ROT
            for sg, (kind, hh, k) in enumerate(seq):
                if last and sg >= n_last:
                    break
                kv_wait(kind, hh, k)
                nk, nh, ni = kv_ahead(kind, hh, k)
                if not (last and nk == "k" and kind == "v"):
                    kv_start(nk, nh, ni)
                elif ni == 0:
                    _copy(wo_hbm.at[pl.ds(h * DH, DH), :], wo_v.at[h], sem_o.at[0]).start(priority=1)
                if not static:
                    if sg < NQ:
                        wq_copy((h + 2) // 2, (h % 2) * (D // 2) + sg * WQ_R, WQ_R).start(priority=0)
                    elif sg < NQ + NO:
                        wo_copy(h + 1, sg - NQ, WO_R).start(priority=0)
                if sg in comp:
                    comp[sg]()
            if last:
                fin()
                wo_wait()
                oproj()
            return st["acc"]

        acc = lax.fori_loop(0, H - 2, head, jnp.zeros((1, D), jnp.float32))
        acc = head(H - 2, acc)
        acc = head(H - 1, acc)

        out_ref[...] = (x + acc * g).astype(out_ref.dtype)

    return kernel


@jax.jit
def pallas_recurrent_scan__sliding_block_cached__glu_gated_swiglu__decode_kernel(
    A_x: jax.Array,
    A_k_cache: jax.Array,
    A_v_cache: jax.Array,
    A_wq: jax.Array,
    A_wo: jax.Array,
    B_x: jax.Array,
    B_w1: jax.Array,
    B_w3: jax.Array,
    B_w2: jax.Array,
):
    B, Sq, D = A_x.shape
    _, H, SK, DH = A_k_cache.shape
    F = B_w1.shape[1]
    assert B == 1 and Sq == 1 and H == _HQ and DH == _DH
    W = min(4096, max(256, SK // 4))

    kt = jnp.swapaxes(A_k_cache, 2, 3)
    vt = jnp.swapaxes(A_v_cache, 2, 3)
    x2 = A_x.reshape(1, D)
    w1 = B_w1.reshape(4, D // 4, F)
    w3 = B_w3.reshape(4, D // 4, F)
    w2 = B_w2.reshape(4, F // 4, D)

    bf16 = jnp.bfloat16
    dma = pltpu.SemaphoreType.DMA
    any_spec = pl.BlockSpec(memory_space=pl.ANY)
    out = pl.pallas_call(
        _make_kernel(D, F, H, SK, W),
        out_shape=jax.ShapeDtypeStruct((1, D), bf16),
        in_specs=[any_spec] * 8,
        out_specs=pl.BlockSpec(memory_space=pltpu.VMEM),
        scratch_shapes=[
            pltpu.VMEM((1, D), bf16),
            pltpu.VMEM((H // 2, D, 2 * DH), bf16),
            pltpu.VMEM((H, DH, D), bf16),
            pltpu.VMEM((4, D // 4, F), bf16),
            pltpu.VMEM((4, D // 4, F), bf16),
            pltpu.VMEM((4, F // 4, D), bf16),
            pltpu.VMEM((DH, W), bf16),
            pltpu.VMEM((DH, W), bf16),
            pltpu.VMEM((H, DH), jnp.float32),
            dma((1,)), dma((3,)), dma((1,)), dma((1,)),
            dma((4,)), dma((4,)), dma((4,)), dma((4,)),
        ],
        compiler_params=pltpu.CompilerParams(
            vmem_limit_bytes=64 * 1024 * 1024,
            disable_bounds_checks=True,
            disable_semaphore_checks=True),
    )(x2, kt, vt, A_wq, A_wo, w1, w3, w2)
    return out.reshape(B, Sq, D)
```

```python
import jax
import jax.numpy as jnp
from jax import lax
import jax.experimental.pallas as pl
import jax.experimental.pallas.tpu as pltpu

_HQ = 32
_DH = 192
_EPS = 1e-5

_RC = 32
_COLS = (0, 1024, 1792, 2560, 3328, 4096)
_LA = 24
_LA_A = 16
_CW = 512
_SM = 8
_WQ_R = 8
_WO_R = 8
_ROT = 7
_SCHED = None

_NN = (((1,), (0,)), ((), ()))
_NT = (((1,), (1,)), ((), ()))


def _silu(x):
    return x * jax.nn.sigmoid(x)


def _dot(a, b, dims=_NN):
    return lax.dot_general(a, b, dims, preferred_element_type=jnp.float32)


def _copy(src, dst, sem):
    return pltpu.make_async_copy(src, dst, sem)


def _wait_region(ref, sem):
    pltpu.make_async_copy(ref, ref, sem).wait()


def _schedule(npc, rot, ready, last_wq):
    n = 2 * npc
    nch = len(ready)
    gap = n // 20
    pos = {}
    used = set()

    def put(name, earliest):
        p = earliest
        while p in used:
            p += 1
        used.add(p)
        pos[name] = p
        return p

    p = -gap
    for j in range(nch):
        p = put(("qk", j), max(ready[j] - rot, p + gap, 0))
    p = put("smax", p + 2)
    p = put("sexp", p + 1)
    p += 2 - gap
    for j in range(nch):
        p = put(("pv", j), max(npc + ready[j] - rot, p + gap))
    p = put("fin", p + 2)
    p = put("oproj", p + 2)
    assert p < n, (p, n)
    return pos


def _make_kernel(D, F, H, SK, W):
    DH = _DH
    LA = _LA
    NR = DH // _RC
    NC = len(_COLS) - 1
    NCH = W // _CW
    NPC = NR * NC
    NST = 2 * NPC
    PW = 2 * DH
    scale = DH ** -0.5
    assert _COLS[-1] == W and LA <= NPC and NCH == 8

    cc_of = [max(c for c in range(NC) if _COLS[c] < (j + 1) * _CW) for j in range(NCH)]
    ready = [NR * (cc_of[j] + 1) - 1 for j in range(NCH)]

    A = 4
    W1_R = 8
    W2_R = 16
    WQ_R = _WQ_R
    NQ = D // 2 // WQ_R
    WO_R = _WO_R
    NO = DH // WO_R
    ROT = _ROT
    NEV = NQ + NO
    ev_at = {}
    for i in range(NEV):
        ev_at.setdefault((i * NST) // NEV, []).append(i)
    last_wq = ((NQ - 1) * NST) // NEV
    first_wo = (NQ * NST) // NEV

    sched = dict(_SCHED) if _SCHED else _schedule(NPC, ROT, ready, last_wq)
    taken = set(sched.values())
    if "qproj" not in sched:
        p = last_wq + max(6, NST // 10)
        while p in taken or (p - 1) in taken:
            p += 1
        sched["qproj"] = p
    sched.setdefault("wowait", first_wo - 1)
    assert sched["qproj"] < NST and sched["wowait"] < first_wo

    def kernel(x_hbm, kt_hbm, vt_hbm, wq_hbm, wo_hbm, w1_hbm, w3_hbm, w2_hbm,
               out_ref,
               x_v, wq_v, wo_v, w1_v, w3_v, w2_v, kbuf, vbuf, q_scr,
               sem_x, sem_w, sem_q, sem_o, sem_k, sem_ks, sem_v, sem_vs):

        def is_split(kind, h, k):
            if not isinstance(h, int) or h < H - 2:
                return False
            if h == H - 2:
                return kind == "v" and k + NPC - LA >= ROT
            return True

        def kv_copy(kind, h, k, part):
            hbm, buf = (kt_hbm, kbuf) if kind == "k" else (vt_hbm, vbuf)
            c, r = divmod(k, NR)
            c0, cw = _COLS[c], _COLS[c + 1] - _COLS[c]
            if part == "full":
                rows, sem = pl.ds(r * _RC, _RC), (sem_k if kind == "k" else sem_v)
            elif part == "bulk":
                rows, sem = pl.ds(r * _RC, _RC - _SM), (sem_k if kind == "k" else sem_v)
            else:
                rows, sem = pl.ds(r * _RC + _RC - _SM, _SM), (sem_ks if kind == "k" else sem_vs)
            return _copy(hbm.at[0, h, rows, pl.ds(SK - W + c0, cw)], buf.at[rows, pl.ds(c0, cw)], sem.at[c])

        def kv_start(kind, h, k):
            if is_split(kind, h, k):
                kv_copy(kind, h, k, "bulk").start(priority=1)
                kv_copy(kind, h, k, "small").start(priority=0)
            else:
                kv_copy(kind, h, k, "full").start(priority=1)

        def kv_wait(kind, h, k):
            kv_copy(kind, h, k, "bulk" if is_split(kind, h, k) else "full").wait()

        def kv_wait_small(kind, h, j):
            lo = cc_of[j - 1] + 1 if j else 0
            for k in range(lo * NR, (cc_of[j] + 1) * NR):
                if is_split(kind, h, k):
                    kv_copy(kind, h, k, "small").wait()

        def kv_ahead(kind, h, k):
            k2 = k + LA
            if k2 < NPC:
                return kind, h, k2
            if kind == "k":
                return "v", h, k2 - NPC
            return "k", h + 1, k2 - NPC

        def wq_copy(p, r0, n):
            c0 = p * PW
            if not isinstance(r0, int):
                r0 = pl.multiple_of(r0, 8)
                c0 = pl.multiple_of(c0, 128)
            return _copy(wq_hbm.at[pl.ds(r0, n), pl.ds(c0, PW)], wq_v.at[p, pl.ds(r0, n), :], sem_q.at[0])

        def wo_copy(h, j, n):
            r0 = h * DH + j * n
            if not isinstance(r0, int):
                r0 = pl.multiple_of(r0, 8)
            return _copy(wo_hbm.at[pl.ds(r0, n), :], wo_v.at[h, pl.ds(j * n, n), :], sem_o.at[0])

        a_steps = []
        for j in range(D // A // W1_R):
            rows = pl.ds(j * W1_R, W1_R)
            a_steps.append(_copy(w1_hbm.at[:, rows, :], w1_v.at[:, rows, :], sem_w.at[0]))
        t_w3 = len(a_steps)
        for j in range(D // A // W1_R):
            rows = pl.ds(j * W1_R, W1_R)
            a_steps.append(_copy(w3_hbm.at[:, rows, :], w3_v.at[:, rows, :], sem_w.at[1]))
        t_w2 = len(a_steps)
        for j in range(F // A // W2_R):
            rows = pl.ds(j * W2_R, W2_R)
            a_steps.append(_copy(w2_hbm.at[:, rows, :], w2_v.at[:, rows, :], sem_w.at[2]))
        n_a = len(a_steps)

        a_small = [wq_copy(0, j * 16, 16) for j in range(D // 16)]
        a_small += [wo_copy(0, j, 8) for j in range(DH // 8)]
        assert len(a_small) == n_a

        cx = _copy(x_hbm, x_v, sem_x.at[0])
        cx.start()
        for t in range(_LA_A):
            a_steps[t].start(priority=1)

        vals = {}

        def do_ln():
            cx.wait()
            x = x_v[...].astype(jnp.float32)
            mu = jnp.mean(x, axis=-1, keepdims=True)
            xc = x - mu
            var = jnp.mean(xc * xc, axis=-1, keepdims=True)
            vals["x"] = x
            vals["xn"] = (xc / jnp.sqrt(var + _EPS)).astype(jnp.bfloat16)

        def q_proj(p):
            _wait_region(wq_v.at[p], sem_q.at[0])
            qp = _dot(vals["xn"], wq_v[p])
            q_scr[pl.ds(2 * p, 1), :] = qp[:, :DH]
            q_scr[pl.ds(2 * p + 1, 1), :] = qp[:, DH:]

        NFC = F // PW

        def do_gate(c):
            w = w1_v[:, :, c * PW:(c + 1) * PW].reshape(D, PW)
            vals["gate", c] = _dot(vals["xn"], w)

        def do_up(c):
            w = w3_v[:, :, c * PW:(c + 1) * PW].reshape(D, PW)
            up = _dot(vals["xn"], w)
            vals["hh", c] = (_silu(vals["gate", c]) * up).astype(jnp.bfloat16)

        def do_ffn(a):
            if a == 0:
                vals["hh"] = jnp.concatenate([vals["hh", c] for c in range(NFC)], axis=1)
            rows = F // A
            part = _dot(vals["hh"][:, a * rows:(a + 1) * rows], w2_v[a])
            vals["ffn"] = part if a == 0 else vals["ffn"] + part

        work = {t: [] for t in range(n_a + ROT)}
        work[0].append(do_ln)
        for c in range(NFC):
            work[t_w3 + c].append(lambda c=c: do_gate(c))
        for c in range(NFC):
            work[t_w2 + c].append(lambda c=c: do_up(c))
        work[t_w2 + 6].append(lambda: q_proj(0))
        for a in range(A):
            work[n_a + (a * ROT) // A].append(lambda a=a: do_ffn(a))

        k0_at = {t: [] for t in range(n_a)}
        for k in range(LA):
            k0_at[n_a - _LA_A + (k * _LA_A) // LA].append(k)
        for t in range(n_a):
            a_steps[t].wait()
            if t + _LA_A < n_a:
                a_steps[t + _LA_A].start(priority=1)
            for k in k0_at[t]:
                kv_start("k", 0, k)
            a_small[t].start(priority=0)
            for fn in work[t]:
                fn()
        for k in range(ROT):
            kv_wait("k", 0, k)
            kv_start(*kv_ahead("k", 0, k))
            for fn in work[n_a + k]:
                fn()

        x = vals["x"]
        g = _silu(vals["ffn"])

        row = lax.broadcasted_iota(jnp.int32, (8, 1), 0)

        def head(h, acc):
            static = isinstance(h, int)
            last = static and h == H - 1
            st = {}

            def qk(j):
                def f():
                    kv_wait_small("k", h, j)
                    if j == 0:
                        q = q_scr[pl.ds(h, 1), :].astype(jnp.bfloat16)
                        st["q8"] = jnp.broadcast_to(q, (8, DH))
                        st["s"] = jnp.zeros((8, _CW), jnp.float32)
                    res = _dot(st["q8"], kbuf[:, j * _CW:(j + 1) * _CW])
                    st["s"] = jnp.where(row == j, res, st["s"])
                return f

            def smax():
                s = st["s"] * scale
                st["s"] = s
                st["m"] = jnp.max(jnp.max(s, axis=1, keepdims=True), axis=0, keepdims=True)

            def sexp():
                p = jnp.exp(st["s"] - st["m"])
                st["l"] = jnp.sum(jnp.sum(p, axis=1, keepdims=True), axis=0, keepdims=True)
                st["pb"] = p.astype(jnp.bfloat16)
                st["o"] = jnp.zeros((8, DH), jnp.float32)

            def pv(j):
                def f():
                    kv_wait_small("v", h, j)
                    res = _dot(st["pb"], vbuf[:, j * _CW:(j + 1) * _CW], _NT)
                    st["o"] = st["o"] + jnp.where(row == j, res, 0.0)
                return f

            def fin():
                o = jnp.sum(st["o"], axis=0, keepdims=True) / st["l"]
                st["ob"] = o.astype(jnp.bfloat16)

            def wo_wait():
                _wait_region(wo_v.at[h], sem_o.at[0])

            def oproj():
                st["acc"] = acc + _dot(st["ob"], wo_v[h])

            def qproj():
                if not static:
                    pl.when(h % 2 == 1)(lambda: q_proj((h + 1) // 2))

            nk = NPC - ROT
            if not last:
                items = [(sched["wowait"], wo_wait)]
                items += [(sched["qk", j], qk(j)) for j in range(NCH)]
                items += [(sched["smax"], smax), (sched["sexp"], sexp)]
                items += [(sched["pv", j], pv(j)) for j in range(NCH)]
                items += [(sched["fin"], fin), (sched["oproj"], oproj), (sched["qproj"], qproj)]
            else:
                items = [(min(sched["qk", j], nk - 1), qk(j)) for j in range(NCH)]
                items += [(nk, smax), (nk, sexp)]
                items += [(nk + ready[j], pv(j)) for j in range(NCH)]
            comp = {}
            for pos, fn in items:
                comp.setdefault(pos, []).append(fn)

            seq = ([("k", h, k) for k in range(ROT, NPC)] + [("v", h, k) for k in range(NPC)]
                   + [("k", h + 1, k) for k in range(ROT)])
            if last:
                seq = seq[:NST - ROT]
            for sg, (kind, hh, k) in enumerate(seq):
                kv_wait(kind, hh, k)
                nkind, nh, ni = kv_ahead(kind, hh, k)
                if not (last and nkind == "k" and kind == "v"):
                    kv_start(nkind, nh, ni)
                elif ni == 0:
                    _copy(wo_hbm.at[pl.ds(h * DH, DH), :], wo_v.at[h], sem_o.at[0]).start(priority=1)
                if not static:
                    for i in ev_at.get(sg, ()):
                        if i < NQ:
                            wq_copy((h + 2) // 2, (h % 2) * (D // 2) + i * WQ_R, WQ_R).start(priority=0)
                        else:
                            wo_copy(h + 1, i - NQ, WO_R).start(priority=0)
                for fn in comp.get(sg, ()):
                    fn()
            if last:
                fin()
                wo_wait()
                oproj()
            return st["acc"]

        acc = lax.fori_loop(0, H - 2, head, jnp.zeros((1, D), jnp.float32))
        acc = head(H - 2, acc)
        acc = head(H - 1, acc)

        out_ref[...] = (x + acc * g).astype(out_ref.dtype)

    return kernel


@jax.jit
def pallas_recurrent_scan__sliding_block_cached__glu_gated_swiglu__decode_kernel(
    A_x: jax.Array,
    A_k_cache: jax.Array,
    A_v_cache: jax.Array,
    A_wq: jax.Array,
    A_wo: jax.Array,
    B_x: jax.Array,
    B_w1: jax.Array,
    B_w3: jax.Array,
    B_w2: jax.Array,
):
    B, Sq, D = A_x.shape
    _, H, SK, DH = A_k_cache.shape
    F = B_w1.shape[1]
    assert B == 1 and Sq == 1 and H == _HQ and DH == _DH
    W = min(4096, max(256, SK // 4))

    kt = jnp.swapaxes(A_k_cache, 2, 3)
    vt = jnp.swapaxes(A_v_cache, 2, 3)
    x2 = A_x.reshape(1, D)
    w1 = B_w1.reshape(4, D // 4, F)
    w3 = B_w3.reshape(4, D // 4, F)
    w2 = B_w2.reshape(4, F // 4, D)

    bf16 = jnp.bfloat16
    dma = pltpu.SemaphoreType.DMA
    nc = len(_COLS) - 1
    any_spec = pl.BlockSpec(memory_space=pl.ANY)
    out = pl.pallas_call(
        _make_kernel(D, F, H, SK, W),
        out_shape=jax.ShapeDtypeStruct((1, D), bf16),
        in_specs=[any_spec] * 8,
        out_specs=pl.BlockSpec(memory_space=pltpu.VMEM),
        scratch_shapes=[
            pltpu.VMEM((1, D), bf16),
            pltpu.VMEM((H // 2, D, 2 * DH), bf16),
            pltpu.VMEM((H, DH, D), bf16),
            pltpu.VMEM((4, D // 4, F), bf16),
            pltpu.VMEM((4, D // 4, F), bf16),
            pltpu.VMEM((4, F // 4, D), bf16),
            pltpu.VMEM((DH, W), bf16),
            pltpu.VMEM((DH, W), bf16),
            pltpu.VMEM((H, DH), jnp.float32),
            dma((1,)), dma((3,)), dma((1,)), dma((1,)),
            dma((nc,)), dma((nc,)), dma((nc,)), dma((nc,)),
        ],
        compiler_params=pltpu.CompilerParams(
            vmem_limit_bytes=64 * 1024 * 1024,
            disable_bounds_checks=True,
            disable_semaphore_checks=True),
    )(x2, kt, vt, A_wq, A_wo, w1, w3, w2)
    return out.reshape(B, Sq, D)
```

```python
import jax
import jax.numpy as jnp
from jax import lax
import jax.experimental.pallas as pl
import jax.experimental.pallas.tpu as pltpu

_HQ = 32
_DH = 192
_EPS = 1e-5

_RC = 32
_COLS = (0, 1024, 1792, 2560, 3328, 4096)
_LA = 24
_LA_A = 16
_CW = 512
_SM = 8
_WQ_R = 8
_WO_R = 8
_ROT = 7
_R2 = 256
_W2_TAIL = (0, 64, 128, 176, 208, 240, 256)
_SCHED = None

_NN = (((1,), (0,)), ((), ()))
_NT = (((1,), (1,)), ((), ()))


def _silu(x):
    return x * jax.nn.sigmoid(x)


def _dot(a, b, dims=_NN):
    return lax.dot_general(a, b, dims, preferred_element_type=jnp.float32)


def _copy(src, dst, sem):
    return pltpu.make_async_copy(src, dst, sem)


def _wait_region(ref, sem):
    pltpu.make_async_copy(ref, ref, sem).wait()


def _schedule(npc, rot, ready, last_wq):
    n = 2 * npc
    nch = len(ready)
    gap = n // 20
    pos = {}
    used = set()

    def put(name, earliest):
        p = earliest
        while p in used:
            p += 1
        used.add(p)
        pos[name] = p
        return p

    p = -gap
    for j in range(nch):
        p = put(("qk", j), max(ready[j] - rot, p + gap, 0))
    p = put("smax", p + 2)
    p = put("sexp", p + 1)
    p += 2 - gap
    for j in range(nch):
        p = put(("pv", j), max(npc + ready[j] - rot, p + gap))
    p = put("fin", p + 2)
    p = put("oproj", p + 2)
    assert p < n, (p, n)
    return pos


def _make_kernel(D, F, H, SK, W):
    DH = _DH
    LA = _LA
    NR = DH // _RC
    NC = len(_COLS) - 1
    NCH = W // _CW
    NPC = NR * NC
    NST = 2 * NPC
    PW = 2 * DH
    scale = DH ** -0.5
    assert _COLS[-1] == W and LA <= NPC and NCH == 8
    assert _W2_TAIL[-1] == _R2 and _R2 % 128 == 0 and _R2 <= F // 4

    cc_of = [max(c for c in range(NC) if _COLS[c] < (j + 1) * _CW) for j in range(NCH)]
    ready = [NR * (cc_of[j] + 1) - 1 for j in range(NCH)]

    A = 4
    W1_R = 8
    W2_R = 16
    WQ_R = _WQ_R
    NQ = D // 2 // WQ_R
    WO_R = _WO_R
    NO = DH // WO_R
    ROT = _ROT
    NEV = NQ + NO
    ev_at = {}
    for i in range(NEV):
        ev_at.setdefault((i * NST) // NEV, []).append(i)
    last_wq = ((NQ - 1) * NST) // NEV
    first_wo = (NQ * NST) // NEV

    sched = dict(_SCHED) if _SCHED else _schedule(NPC, ROT, ready, last_wq)
    taken = set(sched.values())
    if "qproj" not in sched:
        p = last_wq + max(6, NST // 10)
        while p in taken or (p - 1) in taken:
            p += 1
        sched["qproj"] = p
    sched.setdefault("wowait", first_wo - 1)
    assert sched["qproj"] < NST and sched["wowait"] < first_wo

    def kernel(x_hbm, kt_hbm, vt_hbm, wq_hbm, wo_hbm, w1_hbm, w3_hbm, w2_hbm,
               out_ref,
               x_v, wq_v, wo_v, w1_v, w3_v, w2_v, kbuf, vbuf, q_scr, hcol,
               sem_x, sem_w, sem_q, sem_o, sem_t, sem_k, sem_ks, sem_v, sem_vs):

        def is_split(kind, h, k):
            if not isinstance(h, int) or h < H - 2:
                return False
            if h == H - 2:
                return kind == "v" and k + NPC - LA >= ROT
            return True

        def kv_copy(kind, h, k, part):
            hbm, buf = (kt_hbm, kbuf) if kind == "k" else (vt_hbm, vbuf)
            c, r = divmod(k, NR)
            c0, cw = _COLS[c], _COLS[c + 1] - _COLS[c]
            if part == "full":
                rows, sem = pl.ds(r * _RC, _RC), (sem_k if kind == "k" else sem_v)
            elif part == "bulk":
                rows, sem = pl.ds(r * _RC, _RC - _SM), (sem_k if kind == "k" else sem_v)
            else:
                rows, sem = pl.ds(r * _RC + _RC - _SM, _SM), (sem_ks if kind == "k" else sem_vs)
            return _copy(hbm.at[0, h, rows, pl.ds(SK - W + c0, cw)], buf.at[rows, pl.ds(c0, cw)], sem.at[c])

        def kv_start(kind, h, k):
            if is_split(kind, h, k):
                kv_copy(kind, h, k, "bulk").start(priority=1)
                kv_copy(kind, h, k, "small").start(priority=0)
            else:
                kv_copy(kind, h, k, "full").start(priority=1)

        def kv_wait(kind, h, k):
            kv_copy(kind, h, k, "bulk" if is_split(kind, h, k) else "full").wait()

        def kv_wait_small(kind, h, j):
            lo = cc_of[j - 1] + 1 if j else 0
            for k in range(lo * NR, (cc_of[j] + 1) * NR):
                if is_split(kind, h, k):
                    kv_copy(kind, h, k, "small").wait()

        def kv_ahead(kind, h, k):
            k2 = k + LA
            if k2 < NPC:
                return kind, h, k2
            if kind == "k":
                return "v", h, k2 - NPC
            return "k", h + 1, k2 - NPC

        def wq_copy(p, r0, n):
            c0 = p * PW
            if not isinstance(r0, int):
                r0 = pl.multiple_of(r0, 8)
                c0 = pl.multiple_of(c0, 128)
            return _copy(wq_hbm.at[pl.ds(r0, n), pl.ds(c0, PW)], wq_v.at[p, pl.ds(r0, n), :], sem_q.at[0])

        def wo_copy(h, j, n):
            r0 = h * DH + j * n
            if not isinstance(r0, int):
                r0 = pl.multiple_of(r0, 8)
            return _copy(wo_hbm.at[pl.ds(r0, n), :], wo_v.at[h, pl.ds(j * n, n), :], sem_o.at[0])

        a_steps = []
        for j in range(D // A // W1_R):
            rows = pl.ds(j * W1_R, W1_R)
            a_steps.append(_copy(w1_hbm.at[:, rows, :], w1_v.at[:, rows, :], sem_w.at[0]))
        t_w3 = len(a_steps)
        for j in range(D // A // W1_R):
            rows = pl.ds(j * W1_R, W1_R)
            a_steps.append(_copy(w3_hbm.at[:, rows, :], w3_v.at[:, rows, :], sem_w.at[1]))
        t_w2 = len(a_steps)
        T0 = F // A - _R2
        for j in range(F // A // W2_R):
            rows = pl.ds(j * W2_R, W2_R)
            blk = pl.ds(0, A if (j + 1) * W2_R <= T0 else A - 1)
            a_steps.append(_copy(w2_hbm.at[blk, rows, :], w2_v.at[blk, rows, :], sem_w.at[2]))
        NT = len(_W2_TAIL) - 1

        def w2_tail_copy(i):
            rows = pl.ds(T0 + _W2_TAIL[i], _W2_TAIL[i + 1] - _W2_TAIL[i])
            return _copy(w2_hbm.at[A - 1, rows, :], w2_v.at[A - 1, rows, :], sem_t.at[i])
        n_a = len(a_steps)

        a_small = [wq_copy(0, j * 16, 16) for j in range(D // 16)]
        a_small += [wo_copy(0, j, 8) for j in range(DH // 8)]
        assert len(a_small) == n_a

        cx = _copy(x_hbm, x_v, sem_x.at[0])
        cx.start()
        for t in range(_LA_A):
            a_steps[t].start(priority=1)

        vals = {}

        def do_ln():
            cx.wait()
            x = x_v[...].astype(jnp.float32)
            mu = jnp.mean(x, axis=-1, keepdims=True)
            xc = x - mu
            var = jnp.mean(xc * xc, axis=-1, keepdims=True)
            vals["x"] = x
            vals["xn"] = (xc / jnp.sqrt(var + _EPS)).astype(jnp.bfloat16)

        def q_proj(p):
            _wait_region(wq_v.at[p], sem_q.at[0])
            qp = _dot(vals["xn"], wq_v[p])
            q_scr[pl.ds(2 * p, 1), :] = qp[:, :DH]
            q_scr[pl.ds(2 * p + 1, 1), :] = qp[:, DH:]

        NFC = F // PW

        def do_gate(c):
            w = w1_v[:, :, c * PW:(c + 1) * PW].reshape(D, PW)
            vals["gate", c] = _dot(vals["xn"], w)

        def do_up(c):
            w = w3_v[:, :, c * PW:(c + 1) * PW].reshape(D, PW)
            up = _dot(vals["xn"], w)
            vals["hh", c] = (_silu(vals["gate", c]) * up).astype(jnp.bfloat16)

        def do_ffn(a):
            if a == 0:
                vals["hh"] = jnp.concatenate([vals["hh", c] for c in range(NFC)], axis=1)
            rows = F // A
            if a < A - 1:
                part = _dot(vals["hh"][:, a * rows:(a + 1) * rows], w2_v[a])
                vals["ffn"] = part if a == 0 else vals["ffn"] + part
                return
            if T0:
                vals["ffn"] = vals["ffn"] + _dot(vals["hh"][:, a * rows:a * rows + T0], w2_v[a, :T0, :])
            for b in range(_R2 // 128):
                seg = vals["hh"][:, F - _R2 + b * 128:F - _R2 + (b + 1) * 128].astype(jnp.float32)
                hcol[b * 128:(b + 1) * 128, :] = jnp.broadcast_to(seg, (128, 128)).T

        def ffn_rows(i):
            r0, r1 = _W2_TAIL[i], _W2_TAIL[i + 1]
            w2_tail_copy(i).wait()
            w = w2_v[A - 1, T0 + r0:T0 + r1, :].astype(jnp.float32)
            prod = w * jnp.concatenate([hcol[r0:r1, :]] * (D // 128), axis=1)
            part = jnp.sum(prod.reshape((r1 - r0) // 8, 8, D), axis=0)
            vals["tail"] = part if i == 0 else vals["tail"] + part

        work = {t: [] for t in range(n_a + ROT)}
        work[0].append(do_ln)
        for c in range(NFC):
            work[t_w3 + c].append(lambda c=c: do_gate(c))
        for c in range(NFC):
            work[t_w2 + c].append(lambda c=c: do_up(c))
        work[t_w2 + 6].append(lambda: q_proj(0))
        for a in range(A):
            work[n_a + (a * ROT) // A].append(lambda a=a: do_ffn(a))

        k0_at = {t: [] for t in range(n_a)}
        for k in range(LA):
            k0_at[n_a - _LA_A + (k * _LA_A) // LA].append(k)
        for t in range(n_a):
            a_steps[t].wait()
            if t + _LA_A < n_a:
                a_steps[t + _LA_A].start(priority=1)
            for k in k0_at[t]:
                kv_start("k", 0, k)
            a_small[t].start(priority=0)
            for fn in work[t]:
                fn()
        for k in range(ROT):
            kv_wait("k", 0, k)
            kv_start(*kv_ahead("k", 0, k))
            for fn in work[n_a + k]:
                fn()

        x = vals["x"]

        row = lax.broadcasted_iota(jnp.int32, (8, 1), 0)

        def head(h, acc):
            static = isinstance(h, int)
            last = static and h == H - 1
            st = {}

            def qk(j):
                def f():
                    kv_wait_small("k", h, j)
                    if j == 0:
                        q = q_scr[pl.ds(h, 1), :].astype(jnp.bfloat16)
                        st["q8"] = jnp.broadcast_to(q, (8, DH))
                        st["s"] = jnp.zeros((8, _CW), jnp.float32)
                    res = _dot(st["q8"], kbuf[:, j * _CW:(j + 1) * _CW])
                    st["s"] = jnp.where(row == j, res, st["s"])
                return f

            def smax():
                s = st["s"] * scale
                st["s"] = s
                st["m"] = jnp.max(jnp.max(s, axis=1, keepdims=True), axis=0, keepdims=True)

            def sexp():
                p = jnp.exp(st["s"] - st["m"])
                st["l"] = jnp.sum(jnp.sum(p, axis=1, keepdims=True), axis=0, keepdims=True)
                st["pb"] = p.astype(jnp.bfloat16)
                st["o"] = jnp.zeros((8, DH), jnp.float32)

            def pv(j):
                def f():
                    kv_wait_small("v", h, j)
                    res = _dot(st["pb"], vbuf[:, j * _CW:(j + 1) * _CW], _NT)
                    st["o"] = st["o"] + jnp.where(row == j, res, 0.0)
                return f

            def fin():
                o = jnp.sum(st["o"], axis=0, keepdims=True) / st["l"]
                st["ob"] = o.astype(jnp.bfloat16)

            def wo_wait():
                _wait_region(wo_v.at[h], sem_o.at[0])

            def oproj():
                st["acc"] = acc + _dot(st["ob"], wo_v[h])

            def qproj():
                if not static:
                    pl.when(h % 2 == 1)(lambda: q_proj((h + 1) // 2))

            nk = NPC - ROT
            if not last:
                items = [(sched["wowait"], wo_wait)]
                items += [(sched["qk", j], qk(j)) for j in range(NCH)]
                items += [(sched["smax"], smax), (sched["sexp"], sexp)]
                items += [(sched["pv", j], pv(j)) for j in range(NCH)]
                items += [(sched["fin"], fin), (sched["oproj"], oproj), (sched["qproj"], qproj)]
            else:
                items = [(min(sched["qk", j], nk - 1), qk(j)) for j in range(NCH)]
                items += [(nk, smax), (nk, sexp)]
                items += [(nk + ready[j], pv(j)) for j in range(NCH)]
            comp = {}
            for pos, fn in items:
                comp.setdefault(pos, []).append(fn)

            seq = ([("k", h, k) for k in range(ROT, NPC)] + [("v", h, k) for k in range(NPC)]
                   + [("k", h + 1, k) for k in range(ROT)])
            if last:
                seq = seq[:NST - ROT]
            for sg, (kind, hh, k) in enumerate(seq):
                kv_wait(kind, hh, k)
                nkind, nh, ni = kv_ahead(kind, hh, k)
                if not (last and nkind == "k" and kind == "v"):
                    kv_start(nkind, nh, ni)
                elif ni == 0:
                    _copy(wo_hbm.at[pl.ds(h * DH, DH), :], wo_v.at[h], sem_o.at[0]).start(priority=1)
                elif ni <= NT:
                    w2_tail_copy(ni - 1).start(priority=1)
                if not static:
                    for i in ev_at.get(sg, ()):
                        if i < NQ:
                            wq_copy((h + 2) // 2, (h % 2) * (D // 2) + i * WQ_R, WQ_R).start(priority=0)
                        else:
                            wo_copy(h + 1, i - NQ, WO_R).start(priority=0)
                for fn in comp.get(sg, ()):
                    fn()
            if last:
                fin()
                wo_wait()
                oproj()
            return st["acc"]

        acc = lax.fori_loop(0, H - 2, head, jnp.zeros((1, D), jnp.float32))
        acc = head(H - 2, acc)
        acc = head(H - 1, acc)

        for i in range(NT):
            ffn_rows(i)
        g = _silu(vals["ffn"] + jnp.sum(vals["tail"], axis=0, keepdims=True))
        out_ref[...] = (x + acc * g).astype(out_ref.dtype)

    return kernel


@jax.jit
def pallas_recurrent_scan__sliding_block_cached__glu_gated_swiglu__decode_kernel(
    A_x: jax.Array,
    A_k_cache: jax.Array,
    A_v_cache: jax.Array,
    A_wq: jax.Array,
    A_wo: jax.Array,
    B_x: jax.Array,
    B_w1: jax.Array,
    B_w3: jax.Array,
    B_w2: jax.Array,
):
    B, Sq, D = A_x.shape
    _, H, SK, DH = A_k_cache.shape
    F = B_w1.shape[1]
    assert B == 1 and Sq == 1 and H == _HQ and DH == _DH
    W = min(4096, max(256, SK // 4))

    kt = jnp.swapaxes(A_k_cache, 2, 3)
    vt = jnp.swapaxes(A_v_cache, 2, 3)
    x2 = A_x.reshape(1, D)
    w1 = B_w1.reshape(4, D // 4, F)
    w3 = B_w3.reshape(4, D // 4, F)
    w2 = B_w2.reshape(4, F // 4, D)

    bf16 = jnp.bfloat16
    dma = pltpu.SemaphoreType.DMA
    nc = len(_COLS) - 1
    any_spec = pl.BlockSpec(memory_space=pl.ANY)
    out = pl.pallas_call(
        _make_kernel(D, F, H, SK, W),
        out_shape=jax.ShapeDtypeStruct((1, D), bf16),
        in_specs=[any_spec] * 8,
        out_specs=pl.BlockSpec(memory_space=pltpu.VMEM),
        scratch_shapes=[
            pltpu.VMEM((1, D), bf16),
            pltpu.VMEM((H // 2, D, 2 * DH), bf16),
            pltpu.VMEM((H, DH, D), bf16),
            pltpu.VMEM((4, D // 4, F), bf16),
            pltpu.VMEM((4, D // 4, F), bf16),
            pltpu.VMEM((4, F // 4, D), bf16),
            pltpu.VMEM((DH, W), bf16),
            pltpu.VMEM((DH, W), bf16),
            pltpu.VMEM((H, DH), jnp.float32),
            pltpu.VMEM((_R2, 128), jnp.float32),
            dma((1,)), dma((3,)), dma((1,)), dma((1,)),
            dma((len(_W2_TAIL) - 1,)),
            dma((nc,)), dma((nc,)), dma((nc,)), dma((nc,)),
        ],
        compiler_params=pltpu.CompilerParams(
            vmem_limit_bytes=64 * 1024 * 1024,
            disable_bounds_checks=True,
            disable_semaphore_checks=True),
    )(x2, kt, vt, A_wq, A_wo, w1, w3, w2)
    return out.reshape(B, Sq, D)
```
